```python
import os as _os
_os.environ.setdefault('JAX_PLATFORMS', 'cpu')
import jax
import jax.numpy as jnp

def _softmax(x, axis=-1):
    return jax.nn.softmax(x, axis=axis)

def _gelu(x):
    return jax.nn.gelu(x, approximate=True)

def _silu(x):
    return jax.nn.silu(x)

def _sigmoid(x):
    return jax.nn.sigmoid(x)

def _layernorm(x, axis=-1, eps=1e-05):
    m = jnp.mean(x, axis=axis, keepdims=True)
    v = jnp.var(x, axis=axis, keepdims=True)
    return (x - m) / jnp.sqrt(v + eps)

def _scatter_add(tgt, idx, src, axis=0):
    return tgt.at[idx].add(src)

def _segment_sum(src, seg, n):
    return jax.ops.segment_sum(src, seg, n)

class _Rng:

    def __init__(self, key):
        self._k = key

    def _next(self):
        self._k, sub = jax.random.split(self._k)
        return sub

    def normal(self, shape):
        return jax.random.normal(self._next(), shape, dtype=jnp.bfloat16)

    def randint(self, lo, hi, shape):
        return jax.random.randint(self._next(), shape, lo, hi, dtype=jnp.int32)

    def uniform(self, shape, lo=0.0, hi=1.0):
        return jax.random.uniform(self._next(), shape, jnp.bfloat16, lo, hi)

    def permutation(self, n):
        return jax.random.permutation(self._next(), n)
kernel_name = 'adaLN_cond__linear_kernel_hedgehog__geglu_ffn__prompt'

def setup_inputs():
    _rng = _Rng(jax.random.key(int.from_bytes(__import__("os").urandom(4), "little")))
    _w = lambda a: (lambda t: t.astype(jnp.bfloat16) if jnp.issubdtype(t.dtype, jnp.floating) else t)(jnp.asarray(a))

    def _A_setup():
        B, S, D, H = (1, 2048, 512, 32)
        Dh = D // H
        return {'x': _w((lambda *s: _rng.normal(s) * 0.05)(B, S, D)), 'wqkv': _w((lambda *s: _rng.normal(s) * 0.4)(D, 3 * D)), 'w_phi': _w((lambda *s: _rng.normal(s) * 0.4)(H, Dh, Dh) * Dh ** (-0.5)), 'wo': _w((lambda *s: _rng.normal(s) * 0.05)(D, D))}
    _A_in = _A_setup()

    def _B_setup():
        B, S, D, F = (1, 2048, 512, 1792)
        return {'x': _w((lambda *s: _rng.normal(s) * 0.05)(B, S, D)), 'w_gate': _w((lambda *s: _rng.normal(s) * 0.05)(D, F)), 'w_up': _w((lambda *s: _rng.normal(s) * 0.05)(D, F)), 'w_down': _w((lambda *s: _rng.normal(s) * 0.05)(F, D))}
    _B_in = _B_setup()
    return {'A_x': _A_in['x'], 'A_wqkv': _A_in['wqkv'], 'A_w_phi': _A_in['w_phi'], 'A_wo': _A_in['wo'], 'B_x': _B_in['x'], 'B_w_gate': _B_in['w_gate'], 'B_w_up': _B_in['w_up'], 'B_w_down': _B_in['w_down'], 'c': _w((lambda *s: _rng.normal(s) * 0.05)(1, 512) * 8.0), 'w_mod': _w((lambda *s: _rng.normal(s) * 0.05)(512, 6 * 512) * 512 ** (-0.5) * 8.0)}

def reference(A_x, A_wqkv, A_w_phi, A_wo, B_x, B_w_gate, B_w_up, B_w_down, c, w_mod):

    def _A_ref(x, wqkv, w_phi, wo):
        B, S, D = x.shape
        H = 32
        Dh = D // H
        qkv = (lambda x, *d: x.transpose(*d))((x @ wqkv).reshape(B, S, 3, H, Dh), 2, 0, 3, 1, 4)
        q, k, v = (qkv[0], qkv[1], qkv[2])
        pq = jnp.einsum('bhsd,hdf->bhsf', q, w_phi)
        pk = jnp.einsum('bhsd,hdf->bhsf', k, w_phi)
        phi_q = jnp.concatenate([_softmax(pq, axis=-1), _softmax(-pq, axis=-1)], axis=-1)
        phi_k = jnp.concatenate([_softmax(pk, axis=-1), _softmax(-pk, axis=-1)], axis=-1)
        kv = jnp.einsum('bhsf,bhsd->bhfd', phi_k, v)
        z = jnp.einsum('bhsf->bhf', phi_k)
        num = jnp.einsum('bhqf,bhfd->bhqd', phi_q, kv)
        den = jnp.einsum('bhqf,bhf->bhq', phi_q, z)[..., None] + 1e-06
        o = num / den
        return (lambda x, *d: x.transpose(*d))(o, 0, 2, 1, 3).reshape(B, S, D) @ wo

    def _B_ref(x, w_gate, w_up, w_down):
        return _gelu(x @ w_gate) * (x @ w_up) @ w_down
    x = A_x
    mod = (_silu(c) @ w_mod).reshape(c.shape[0], 6, 1, -1)
    sa, ca, ga, sb, cb, gb = (mod[:, 0].copy(), mod[:, 1].copy(), mod[:, 2].copy(), mod[:, 3].copy(), mod[:, 4].copy(), mod[:, 5].copy())
    h = _layernorm(x, axis=-1) * (1 + ca) + sa
    x = x + ga * _A_ref(h, A_wqkv, A_w_phi, A_wo)
    h = _layernorm(x, axis=-1) * (1 + cb) + sb
    x = x + gb * _B_ref(h, B_w_gate, B_w_up, B_w_down)
    return x
```

```python
import numpy as np
import jax
import jax.numpy as jnp
from jax import lax
import jax.experimental.pallas as pl
import jax.experimental.pallas.tpu as pltpu

S, D, H, DH, F = 2048, 512, 32, 16, 1792
G = 4
T1 = 512
T2 = 512
FC = 256
BF = jnp.bfloat16
F32 = jnp.float32
NT = (((1,), (1,)), ((), ()))
TN = (((0,), (0,)), ((), ()))


def _dot(a, b, dn=None):
    if dn is None:
        return jnp.dot(a, b, preferred_element_type=F32)
    return lax.dot_general(a, b, dn, preferred_element_type=F32)


def _ln_mod(x, shift, scale1):
    m = jnp.mean(x, axis=-1, keepdims=True)
    xc = x - m
    v = jnp.mean(xc * xc, axis=-1, keepdims=True)
    return xc * lax.rsqrt(v + 1e-5) * scale1 + shift


def _phi(p):
    sl = [p[f * 8:(f + 1) * 8] for f in range(DH)]
    mx, mn = sl[0], sl[0]
    for s in sl[1:]:
        mx = jnp.maximum(mx, s)
        mn = jnp.minimum(mn, s)
    ep = [jnp.exp(s - mx) for s in sl]
    en = [jnp.exp(mn - s) for s in sl]
    sp, sn = ep[0], en[0]
    for a, b in zip(ep[1:], en[1:]):
        sp = sp + a
        sn = sn + b
    rp, rn = 1.0 / sp, 1.0 / sn
    return jnp.concatenate([e * rp for e in ep] + [e * rn for e in en], axis=0)


def _kernel(x_hbm, wqkv_hbm, wphi_hbm, wo_hbm, wg_hbm, wu_hbm, wd_hbm, c_hbm, wmod_hbm,
            o_hbm,
            x_v, wqkv_v, wphi_v, wo_v, wg_v, wu_v, wd_v, c_v, wmod_v,
            wt_v, wop_v, h_v, kvt_v, z_v, mod_v, o_v, act_v, x1_v, h2_v,
            sem_x, sem_w, sem_o):
    n1, n2 = S // T1, S // T2

    def xcp(i):
        r = pl.ds(i * T1, T1)
        return pltpu.make_async_copy(x_hbm.at[r], x_v.at[r], sem_x.at[i])

    cp_c = pltpu.make_async_copy(c_hbm, c_v, sem_w.at[0])
    cp_phi = pltpu.make_async_copy(wphi_hbm, wphi_v, sem_w.at[1])
    cp_m0 = pltpu.make_async_copy(wmod_hbm.at[:, :2 * D], wmod_v.at[:, :2 * D], sem_w.at[2])
    cp_kv = pltpu.make_async_copy(wqkv_hbm.at[:, D:], wqkv_v.at[:, D:], sem_w.at[3])
    cp_q = pltpu.make_async_copy(wqkv_hbm.at[:, :D], wqkv_v.at[:, :D], sem_w.at[4])
    cp_m1 = pltpu.make_async_copy(wmod_hbm.at[:, 2 * D:], wmod_v.at[:, 2 * D:], sem_w.at[5])
    cp_o = pltpu.make_async_copy(wo_hbm, wo_v, sem_w.at[6])
    cp_g = pltpu.make_async_copy(wg_hbm, wg_v, sem_w.at[7])
    cp_u = pltpu.make_async_copy(wu_hbm, wu_v, sem_w.at[8])
    cp_d = pltpu.make_async_copy(wd_hbm, wd_v, sem_w.at[9])

    for cp in (cp_c, cp_phi, cp_kv, cp_m0, xcp(0)):
        cp.start()

    def iotas(n, m):
        return (lax.broadcasted_iota(jnp.int32, (n, m), 0), lax.broadcasted_iota(jnp.int32, (n, m), 1))

    row, col = iotas(D, H)
    sel = (col == (row // 128) * 8 + row % 8).astype(BF)
    row, col = iotas(D, DH * DH)
    same_f = (col % DH) == ((row // 8) % DH)
    row, col = iotas(DH * DH, 128)
    expand = ((row // DH) == (col % DH)).astype(BF)
    row = lax.broadcasted_iota(jnp.int32, (128, 128), 0)
    col = lax.broadcasted_iota(jnp.int32, (128, 128), 1)
    same_head = (row % 8) == (col // DH)
    perm = jnp.logical_and(same_head, (row // 8) == (col % DH)).astype(BF)
    cp_phi.wait()
    pa = _dot(sel, wphi_v[...].reshape(DH * DH, H), NT)
    pt = _dot(jnp.where(same_f, pa, 0.0).astype(BF), expand)
    bdt = [jnp.where(same_head, pt[g * 128:(g + 1) * 128], 0.0).astype(BF) for g in range(G)]

    cp_kv.wait()
    for g in range(G):
        wk = wqkv_v[:, D + g * 128:D + (g + 1) * 128]
        wt_v[D + g * 128:D + (g + 1) * 128, :] = _dot(bdt[g], wk, NT).astype(BF)
        wv = wqkv_v[:, 2 * D + g * 128:2 * D + (g + 1) * 128]
        wt_v[2 * D + g * 128:2 * D + (g + 1) * 128, :] = _dot(perm, wv, NT).astype(BF)

    cp_c.wait()
    cv = c_v[...].astype(F32)
    sc = jnp.broadcast_to(cv * jax.nn.sigmoid(cv), (128, D)).T

    def mod_cols(lo, hi):
        for j in range(lo, hi):
            cs = slice(j * 128, (j + 1) * 128)
            mod_v[:, cs] = jnp.sum(wmod_v[:, cs].astype(F32) * sc, axis=0, keepdims=True)

    cp_m0.wait()
    for cp in [xcp(i) for i in range(1, n1)]:
        cp.start()
    mod_cols(0, 8)
    kvt_v[...] = jnp.zeros_like(kvt_v)
    z_v[...] = jnp.zeros_like(z_v)

    def p1(i, extra=lambda g: None):
        r = pl.ds(pl.multiple_of(i * T1, T1), T1)
        xcp(i).wait()
        if not isinstance(i, int):
            @pl.when(i == 0)
            def _():
                for cp in (cp_q, cp_m1, cp_o):
                    cp.start()
        h = _ln_mod(x_v[r, :].astype(F32), mod_v[0:1, 0:D], 1.0 + mod_v[0:1, D:2 * D]).astype(BF)
        h_v[r, :] = h
        kv = _dot(wt_v[D:, :], h, NT)
        for g in range(G):
            phi = _phi(kv[g * 128:(g + 1) * 128])
            vt = kv[D + g * 128:D + (g + 1) * 128].astype(BF)
            zs = phi[:, 0:128]
            for j in range(1, T1 // 128):
                zs = zs + phi[:, j * 128:(j + 1) * 128]
            z_v[g] += zs
            kvt_v[g] += _dot(vt, phi.astype(BF), NT)
            extra(g)

    lax.fori_loop(0, n1 - 1, lambda i, _: p1(i), None)
    cp_g.start()
    cp_u.start()
    cp_d.start()
    cp_q.wait()
    cp_m1.wait()
    cp_o.wait()

    def prep2(g):
        gs = slice(g * 128, (g + 1) * 128)
        mod_cols(8 + 4 * g, 12 + 4 * g)
        wt_v[gs, :] = _dot(bdt[g], wqkv_v[:, gs], NT).astype(BF)
        wop_v[gs, :] = _dot(perm, wo_v[gs, :]).astype(BF)

    p1(n1 - 1, prep2)

    def run(kz_v):
        row = lax.broadcasted_iota(jnp.int32, (144, 256), 0)
        col = lax.broadcasted_iota(jnp.int32, (144, 256), 1)
        keep = (row % 8) == (col % 8)
        for g in range(G):
            zt = jnp.sum(z_v[g].T, axis=0, keepdims=True)
            full = jnp.concatenate([kvt_v[g], jnp.broadcast_to(zt, (16, 256))], axis=0)
            kz_v[g] = jnp.where(keep, full, 0.0).astype(BF)

        def attn(i, slot):
            r = pl.ds(pl.multiple_of(i * T2, T2), T2)
            q = _dot(wt_v[:D, :], h_v[r, :], NT)
            yield
            ots = []
            for g in range(G):
                phi = _phi(q[g * 128:(g + 1) * 128]).astype(BF)
                nd = _dot(kz_v[g], phi)
                rd = 1.0 / (nd[128:136] + 1e-6)
                ots += [nd[d * 8:(d + 1) * 8] * rd for d in range(DH)]
                yield
            ot = jnp.concatenate(ots, axis=0).astype(BF)
            a = _dot(ot, wop_v[...], TN)
            yield
            x1 = x_v[r, :].astype(F32) + mod_v[:, 2 * D:3 * D] * a
            x1_v[slot] = x1
            h2_v[slot] = _ln_mod(x1, mod_v[:, 3 * D:4 * D], 1.0 + mod_v[:, 4 * D:5 * D]).astype(BF)

        def ffn(i, slot, other=iter(())):
            r = pl.ds(pl.multiple_of(i * T2, T2), T2)
            h2 = h2_v[slot]
            for j in range(F // FC):
                next(other, None)
                cs = slice(j * FC, (j + 1) * FC)
                gt = _dot(h2, wg_v[:, cs])
                up = _dot(h2, wu_v[:, cs])
                act_v[:, cs] = (jax.nn.gelu(gt, approximate=True) * up).astype(BF)
            hh = T2 // 2
            for m in range(2):
                rm = pl.ds(pl.multiple_of(i * T2 + m * hh, hh), hh)
                y = _dot(act_v[m * hh:(m + 1) * hh, :], wd_v[...])
                o_v[rm, :] = (x1_v[slot, m * hh:(m + 1) * hh, :] + mod_v[:, 5 * D:] * y).astype(BF)
                pltpu.make_async_copy(o_v.at[rm], o_hbm.at[rm], sem_o.at[i]).start()

        for _ in attn(0, 0):
            pass
        cp_g.wait()
        cp_u.wait()
        cp_d.wait()
        lax.fori_loop(0, n2 - 1, lambda i, _: ffn(i, i % 2, attn(i + 1, (i + 1) % 2)), None)
        ffn(n2 - 1, (n2 - 1) % 2)

    pl.run_scoped(run, pltpu.VMEM((G, 144, 256), BF))
    for i in range(n2):
        r = pl.ds(i * T2, T2)
        pltpu.make_async_copy(o_v.at[r], o_hbm.at[r], sem_o.at[i]).wait()


@jax.jit
def pallas_adaLN_cond__linear_kernel_hedgehog__geglu_ffn__prompt_kernel(
    A_x, A_wqkv, A_w_phi, A_wo, B_x, B_w_gate, B_w_up, B_w_down, c, w_mod,
):
    del B_x
    V = pltpu.VMEM
    out = pl.pallas_call(
        _kernel,
        out_shape=jax.ShapeDtypeStruct((S, D), BF),
        in_specs=[pl.BlockSpec(memory_space=pl.ANY)] * 9,
        out_specs=pl.BlockSpec(memory_space=pl.ANY),
        scratch_shapes=[
            V((S, D), BF), V((D, 3 * D), BF), V((DH, DH, H), BF), V((D, D), BF),
            V((D, F), BF), V((D, F), BF), V((F, D), BF), V((1, D), BF), V((D, 6 * D), BF),
            V((3 * D, D), BF), V((D, D), BF), V((S, D), BF),
            V((G, 128, 256), F32), V((G, 256, 128), F32), V((1, 6 * D), F32),
            V((S, D), BF), V((T2, F), BF), V((2, T2, D), F32), V((2, T2, D), BF),
            pltpu.SemaphoreType.DMA((S // T1,)), pltpu.SemaphoreType.DMA((10,)),
            pltpu.SemaphoreType.DMA((S // T2,)),
        ],
        compiler_params=pltpu.CompilerParams(vmem_limit_bytes=100 * 1024 * 1024),
    )(A_x.reshape(S, D), A_wqkv, A_w_phi.transpose(1, 2, 0), A_wo, B_w_gate, B_w_up, B_w_down, c, w_mod)
    return out.reshape(1, S, D)
```
